```python
import jax
import jax.numpy as jnp

def _softmax(x, axis=-1):
    return jax.nn.softmax(x, axis=axis)

def _gelu(x):
    return jax.nn.gelu(x, approximate=True)

def _silu(x):
    return jax.nn.silu(x)

def _sigmoid(x):
    return jax.nn.sigmoid(x)

def _layernorm(x, axis=-1, eps=1e-05):
    m = jnp.mean(x, axis=axis, keepdims=True)
    v = jnp.var(x, axis=axis, keepdims=True)
    return (x - m) / jnp.sqrt(v + eps)

def _scatter_add(tgt, idx, src, axis=0):
    return tgt.at[idx].add(src)

def _segment_sum(src, seg, n):
    return jax.ops.segment_sum(src, seg, n)

class _Rng:

    def __init__(self, key):
        self._k = key

    def _next(self):
        self._k, sub = jax.random.split(self._k)
        return sub

    def normal(self, shape):
        return jax.random.normal(self._next(), shape, dtype=jnp.bfloat16)

    def randint(self, lo, hi, shape):
        return jax.random.randint(self._next(), shape, lo, hi, dtype=jnp.int32)

    def uniform(self, shape, lo=0.0, hi=1.0):
        return jax.random.uniform(self._next(), shape, jnp.bfloat16, lo, hi)

    def permutation(self, n):
        return jax.random.permutation(self._next(), n)
kernel_name = 'adaLN_cond__sliding_block_cached__mixer_s_mlp__decode'

def setup_inputs():
    _rng = _Rng(jax.random.key(int.from_bytes(__import__("os").urandom(4), "little")))
    _w = lambda a: (lambda t: t.astype(jnp.bfloat16) if jnp.issubdtype(t.dtype, jnp.floating) else t)(jnp.asarray(a))

    def _A_setup():
        B, Sq, D = (1, 1, 448)
        Hq, Hkv, Sk, Dh = (16, 8, 65536, 256)
        assert Hq % Hkv == 0, (Hq, Hkv)
        return {'x': _w((lambda *s: _rng.normal(s) * 0.05)(B, Sq, D)), 'k_cache': _w((lambda *s: _rng.normal(s) * 0.05)(B, Hkv, Sk, Dh)), 'v_cache': _w((lambda *s: _rng.normal(s) * 0.05)(B, Hkv, Sk, Dh)), 'wq': _w((lambda *s: _rng.normal(s) * 0.05)(D, Hq * Dh) * D ** (-0.5)), 'wo': _w((lambda *s: _rng.normal(s) * 0.05)(Hq * Dh, D) * (Hq * Dh) ** (-0.5))}
    _A_in = _A_setup()

    def _B_setup():
        B, S, D, F = (1, 1, 448, 1792)
        return {'x': _w((lambda *s: _rng.normal(s) * 0.05)(B, S, D)), 'w1': _w((lambda *s: _rng.normal(s) * 0.05)(D, D) * D ** (-0.5)), 'w2': _w((lambda *s: _rng.normal(s) * 0.05)(D, D) * D ** (-0.5)), 'w3': _w((lambda *s: _rng.normal(s) * 0.05)(D, F) * D ** (-0.5)), 'w4': _w((lambda *s: _rng.normal(s) * 0.05)(F, D) * F ** (-0.5))}
    _B_in = _B_setup()
    return {'A_x': _A_in['x'], 'A_k_cache': _A_in['k_cache'], 'A_v_cache': _A_in['v_cache'], 'A_wq': _A_in['wq'], 'A_wo': _A_in['wo'], 'B_x': _B_in['x'], 'B_w1': _B_in['w1'], 'B_w2': _B_in['w2'], 'B_w3': _B_in['w3'], 'B_w4': _B_in['w4'], 'c': _w((lambda *s: _rng.normal(s) * 0.05)(1, 448)), 'w_mod': _w((lambda *s: _rng.normal(s) * 0.05)(448, 6 * 448) * 448 ** (-0.5))}

def reference(A_x, A_k_cache, A_v_cache, A_wq, A_wo, B_x, B_w1, B_w2, B_w3, B_w4, c, w_mod):

    def _A_ref(x, k_cache, v_cache, wq, wo):
        B, Sq, D = x.shape
        Hq, Dh = (16, 256)
        Hkv, Sk = (k_cache.shape[1], k_cache.shape[2])
        W = min(4096, max(256, Sk // 4))
        rep = Hq // Hkv
        q = (lambda x, *d: x.transpose(*d))((x @ wq).reshape(B, Sq, Hq, Dh), 0, 2, 1, 3)
        k = jnp.repeat(k_cache[:, :, Sk - W:, :], rep, axis=1)
        v = jnp.repeat(v_cache[:, :, Sk - W:, :], rep, axis=1)
        scores = jnp.einsum('bhqd,bhkd->bhqk', q, k) * Dh ** (-0.5)
        p = _softmax(scores, axis=-1)
        o = jnp.einsum('bhqk,bhkd->bhqd', p, v)
        return (lambda x, *d: x.transpose(*d))(o, 0, 2, 1, 3).reshape(B, Sq, Hq * Dh) @ wo

    def _B_ref(x, w1, w2, w3, w4):
        B, S, D = x.shape
        h = _gelu(_layernorm(x, axis=-1) @ w1)
        c = D // 4
        g0 = jnp.pad(h[:, :, 0 * c:1 * c], ((0, 0), (1, 0), (0, 0)))[:, :S, :]
        g1 = jnp.pad(h[:, :, 1 * c:2 * c], ((0, 0), (0, 1), (0, 0)))[:, 1:, :]
        g2 = jnp.pad(h[:, :, 2 * c:3 * c], ((0, 0), (2, 0), (0, 0)))[:, :S, :]
        g3 = jnp.pad(h[:, :, 3 * c:], ((0, 0), (0, 2), (0, 0)))[:, 2:, :]
        hs = jnp.concatenate([g0, g1, g2, g3], axis=-1) @ w2
        x1 = x + hs
        h2 = _gelu(_layernorm(x1, axis=-1) @ w3) @ w4
        return x1 + h2
    x = A_x
    mod = (_silu(c) @ w_mod).reshape(c.shape[0], 6, 1, -1)
    sa, ca, ga, sb, cb, gb = (mod[:, 0].copy(), mod[:, 1].copy(), mod[:, 2].copy(), mod[:, 3].copy(), mod[:, 4].copy(), mod[:, 5].copy())
    h = _layernorm(x, axis=-1) * (1 + ca) + sa
    x = x + ga * _A_ref(h, A_k_cache, A_v_cache, A_wq, A_wo)
    h = _layernorm(x, axis=-1) * (1 + cb) + sb
    x = x + gb * _B_ref(h, B_w1, B_w2, B_w3, B_w4)
    return x
```

```python
import functools
import jax, jax.numpy as jnp
from jax import lax
from jax.experimental import pallas as pl
from jax.experimental.pallas import tpu as pltpu

D, F, HQ, HKV, DH, SK, W = 448, 1792, 16, 8, 256, 65536, 4096
BF, F32 = jnp.bfloat16, jnp.float32
NT = (((1,), (1,)), ((), ()))

DEFAULT = dict(R=128, CH=32, L=3, kvpat=(0, 1, 1, 0), wpat=(0, 1, 1, 0), wspread=True, compute=True)

def _ln(x):
    m = jnp.mean(x, axis=-1, keepdims=True)
    d = x - m
    v = jnp.mean(d * d, axis=-1, keepdims=True)
    return d * lax.rsqrt(v + 1e-5)

def make(**kw):
    cfg = dict(DEFAULT); cfg.update(kw)
    R, CH, L = cfg['R'], cfg['CH'], cfg['L']
    NB = W // R
    do = cfg['compute']

    def kernel(x_hbm, c_hbm, k_hbm, v_hbm, wm_hbm, wq_hbm, wo_hbm, w3_hbm, w4_hbm, o_hbm,
               xb, cb, kb, vb, wmb, wqb, wob, w3b, w4b, qf, sc, ob, wsem, ksem, vsem, ssem):
        def w_issue(src, dst, c0, width, sem):
            def it(i, _):
                for j in range(8):
                    g = (j * 7 + i) if cfg['wspread'] else (i * 8 + j)
                    r0 = pl.multiple_of(g * 8, 8)
                    pltpu.make_async_copy(src.at[pl.ds(r0, 8), pl.ds(c0, width)], dst.at[pl.ds(r0, 8), pl.ds(c0, width)], sem
                                          ).start(priority=cfg['wpat'][j % len(cfg['wpat'])])
            lax.fori_loop(0, 7, it, None)
        def w_wait(dst, c0, width, sem):
            v = dst.at[:, pl.ds(c0, width)]
            pltpu.make_async_copy(v, v, sem).wait()
        def kv_issue(src, dst, i, sem):
            def it(t, _):
                r0 = pl.multiple_of(i * R + t * CH, CH)
                for h in range(HKV):
                    pltpu.make_async_copy(src.at[0, h, pl.ds(SK - W + r0, CH)], dst.at[h, pl.ds(r0, CH)], sem
                                          ).start(priority=cfg['kvpat'][h % len(cfg['kvpat'])])
            lax.fori_loop(0, R // CH, it, None, unroll=cfg.get('kvunroll', True))
        def kv_wait(dst, i, sem):
            v = dst.at[:, pl.ds(pl.multiple_of(i * R, R), R)]
            pltpu.make_async_copy(v, v, sem).wait()

        wblocks = ([(wm_hbm, wmb, 896 * j, 896) for j in range(3)] + [(wq_hbm, wqb, 1024 * j, 1024) for j in range(4)]
                   + [(wo_hbm, wob, 1024 * j, 1024) for j in range(4)] + [(w3_hbm, w3b, 896 * j, 896) for j in range(2)]
                   + [(w4_hbm, w4b, 896 * j, 896) for j in range(2)])
        def wi(j):
            s, d, c0, wd = wblocks[j]
            w_issue(s, d, c0, wd, wsem.at[j])
        def ww(j):
            s, d, c0, wd = wblocks[j]
            w_wait(d, c0, wd, wsem.at[j])

        xcp = pltpu.make_async_copy(x_hbm.at[0], xb, ssem.at[0])
        ccp = pltpu.make_async_copy(c_hbm, cb, ssem.at[1])
        row8 = lax.broadcasted_iota(jnp.int32, (8, 1), 0)

        wi(0)
        ccp.start(); xcp.start()
        wi(1)
        ccp.wait(); xcp.wait()
        if do:
            c = jnp.broadcast_to(cb[...].astype(F32), (8, D))
            s = (c * jax.nn.sigmoid(c)).astype(BF)
            x = jnp.broadcast_to(xb[...].astype(F32), (8, D))
            xn = _ln(x)
        wi(2)
        ww(0)
        if do:
            m0 = jnp.dot(s, wmb[:, 0:896], preferred_element_type=F32)
            h = (xn * (1.0 + m0[:, D:2 * D]) + m0[:, 0:D]).astype(BF)
        wi(3)
        ww(1)
        if do:
            m1 = jnp.dot(s, wmb[:, 896:1792], preferred_element_type=F32)
        wi(4)
        ww(2)
        if do:
            m2 = jnp.dot(s, wmb[:, 1792:2688], preferred_element_type=F32)
        q = [jnp.zeros((8, DH), F32), jnp.zeros((8, DH), F32)]
        for j in range(4):
            if j + 5 <= 6:
                wi(j + 5)
            elif j == 2:
                for i in range(min(2, L)):
                    kv_issue(k_hbm, kb, i, ksem.at[i])
            else:
                for i in range(2, L):
                    kv_issue(k_hbm, kb, i, ksem.at[i])
            ww(3 + j)
            if do:
                r = jnp.dot(h, wqb[:, 1024 * j:1024 * (j + 1)], preferred_element_type=F32)
                for t in range(4):
                    hq = 4 * j + t
                    q[hq // 8] = jnp.where(row8 == hq % 8, r[:, DH * t:DH * (t + 1)], q[hq // 8])
        if do:
            qf[0] = q[0] * (DH ** -0.5)
            qf[1] = q[1] * (DH ** -0.5)

        def k_step(i, mx):
            @pl.when(i + L < NB)
            def _():
                kv_issue(k_hbm, kb, i + L, ksem.at[i + L])
            @pl.when(i + L >= NB)
            def _():
                kv_issue(v_hbm, vb, i + L - NB, vsem.at[i + L - NB])
            kv_wait(kb, i, ksem.at[i])
            if not do:
                return mx
            r0 = pl.multiple_of(i * R, R)
            out = []
            for g in range(2):
                qg = qf[g].astype(BF)
                sg = None
                for j in range(4):
                    r = lax.dot_general(qg, kb[4 * g + j, pl.ds(r0, R), :], NT, preferred_element_type=F32)
                    sg = r if sg is None else jnp.where(row8 // 2 == j, r, sg)
                sc[g, i] = sg
                m = sg[:, 0:128]
                for t in range(1, R // 128):
                    m = jnp.maximum(m, sg[:, 128 * t:128 * (t + 1)])
                out.append(jnp.maximum(mx[g], m))
            return tuple(out)
        ninf = jnp.full((8, 128), -jnp.inf, F32)
        mx = lax.fori_loop(0, NB, k_step, (ninf, ninf))

        if do:
            for g in range(2):
                m = jnp.max(mx[g], axis=-1, keepdims=True)
                e = jnp.exp(sc[g] - m)
                l = jnp.sum(jnp.sum(e, axis=0), axis=-1, keepdims=True)
                sc[g] = e * (1.0 / l)

        def v_step(i, acc):
            @pl.when(i + L < NB)
            def _():
                kv_issue(v_hbm, vb, i + L, vsem.at[i + L])
            @pl.when(i + L == NB)
            def _():
                wi(7)
            @pl.when(i + L == NB + 1)
            def _():
                wi(8)
            kv_wait(vb, i, vsem.at[i])
            if not do:
                return acc
            r0 = pl.multiple_of(i * R, R)
            out = []
            for g in range(2):
                pg = sc[g, i].astype(BF)
                og = None
                for j in range(4):
                    r = jnp.dot(pg, vb[4 * g + j, pl.ds(r0, R), :], preferred_element_type=F32)
                    og = r if og is None else jnp.where(row8 // 2 == j, r, og)
                out.append(acc[g] + og)
            return tuple(out)
        z = jnp.zeros((8, DH), F32)
        o = lax.fori_loop(0, NB, v_step, (z, z))

        acc = jnp.zeros((8, D), F32)
        for j in range(4):
            wi(9 + j)
            ww(7 + j)
            if do:
                lhs = jnp.concatenate([jnp.where(row8 == (4 * j + t) % 8, o[j // 2], 0.0) for t in range(4)], axis=1).astype(BF)
                acc = acc + lax.dot_general(lhs, wob[:, 1024 * j:1024 * (j + 1)], NT, preferred_element_type=F32)
        wi(13)
        if do:
            attn = jnp.sum(acc, axis=0, keepdims=True)
            x1 = x + m1[:, 0:D] * attn
            h2 = _ln(x1) * (1.0 + m2[:, 0:D]) + m1[:, D:2 * D]
            hn = _ln(h2).astype(BF)
        wi(14)
        u = []
        for j in range(2):
            ww(11 + j)
            if do:
                u.append(jax.nn.gelu(jnp.dot(hn, w3b[:, 896 * j:896 * (j + 1)], preferred_element_type=F32), approximate=True).astype(BF))
        if do:
            y = h2
        for j in range(2):
            ww(13 + j)
            if do:
                y = y + lax.dot_general(u[j], w4b[:, 896 * j:896 * (j + 1)], NT, preferred_element_type=F32)
        if do:
            res = x1 + m2[:, D:2 * D] * y
            ob[...] = res[0:1, :].astype(BF)
        else:
            ob[...] = jnp.zeros(ob.shape, BF)
        ocp = pltpu.make_async_copy(ob, o_hbm.at[0], ssem.at[2])
        ocp.start(); ocp.wait()

    def f(A_x, A_k_cache, A_v_cache, A_wq, A_wo, B_x, B_w1, B_w2, B_w3, B_w4, c, w_mod):
        hb = pl.BlockSpec(memory_space=pltpu.HBM)
        args = [A_x, c, A_k_cache, A_v_cache, w_mod, A_wq, A_wo.T, B_w3, B_w4.T]
        args = [pltpu.with_memory_space_constraint(a, pltpu.HBM) for a in args]
        return pl.pallas_call(kernel, in_specs=[hb] * 9, out_specs=hb,
            out_shape=jax.ShapeDtypeStruct((1, 1, D), BF),
            scratch_shapes=[pltpu.VMEM((1, D), BF), pltpu.VMEM((1, D), BF),
                pltpu.VMEM((HKV, W, DH), BF), pltpu.VMEM((HKV, W, DH), BF),
                pltpu.VMEM((D, 6 * D), BF), pltpu.VMEM((D, HQ * DH), BF), pltpu.VMEM((D, HQ * DH), BF),
                pltpu.VMEM((D, F), BF), pltpu.VMEM((D, F), BF),
                pltpu.VMEM((2, 8, DH), F32), pltpu.VMEM((2, NB, 8, R), F32), pltpu.VMEM((1, D), BF),
                pltpu.SemaphoreType.DMA((15,)), pltpu.SemaphoreType.DMA((NB,)), pltpu.SemaphoreType.DMA((NB,)),
                pltpu.SemaphoreType.DMA((3,))],
            compiler_params=pltpu.CompilerParams(vmem_limit_bytes=100 * 2**20, disable_bounds_checks=True, disable_semaphore_checks=True),
        )(*args)
    return f


@jax.jit
def pallas_adaLN_cond__sliding_block_cached__mixer_s_mlp__decode_kernel(
    A_x, A_k_cache, A_v_cache, A_wq, A_wo, B_x, B_w1, B_w2, B_w3, B_w4, c, w_mod):
    return make(wpat=(0, 1))(A_x, A_k_cache, A_v_cache, A_wq, A_wo, B_x, B_w1, B_w2, B_w3, B_w4, c, w_mod)
```

```python
import jax, jax.numpy as jnp
from jax import lax
from jax.experimental import pallas as pl
from jax.experimental.pallas import tpu as pltpu

D, F, HQ, HKV, DH, SK, W = 448, 1792, 16, 8, 256, 65536, 4096
BF, F32 = jnp.bfloat16, jnp.float32
NT = (((1,), (1,)), ((), ()))

DEFAULT = dict(R=256, CH=64, L=3, shift=2, perm=tuple(range(8)), compute=True,
               w4=[(0, 128, 0, 1792, 8), (128, 128, 0, 1792, 8), (256, 128, 0, 1792, 8), (384, 64, 0, 1792, 8)],
               wm=[(0, 448, 0, 1280, 8), (0, 448, 1280, 1408, 8)],
               ns=8, ahead=96, solo=28, lag=28)

def _ln(x):
    m = jnp.mean(x, axis=-1, keepdims=True)
    d = x - m
    v = jnp.mean(d * d, axis=-1, keepdims=True)
    return d * lax.rsqrt(v + 1e-5)

def make(**kw):
    cfg = dict(DEFAULT); cfg.update(kw)
    R, CH, L = cfg['R'], cfg['CH'], cfg['L']
    NB = W // R
    do = cfg['compute']
    skip = cfg.get('skip', '')
    n4, nm = len(cfg['w4']), len(cfg['wm'])

    def kernel(x_hbm, c_hbm, k_hbm, v_hbm, wm_hbm, wq_hbm, wo_hbm, w3_hbm, w4_hbm, o_hbm,
               xb, cb, kb, vb, wmb, wqb, wob, w3b, w4b, sc, modb, qb, accb, ob, wsem, ksem, vsem, ssem):
        blocks = {}
        for j, b in enumerate(cfg['wm']): blocks['m', j] = (wm_hbm, wmb) + b
        for j in range(2): blocks['q', j] = (wq_hbm, wqb, 0, D, 2048 * j, 2048, 8)
        for j in range(2): blocks['o', j] = (wo_hbm, wob, 0, D, 2048 * j, 2048, 8)
        blocks['3', 0] = (w3_hbm, w3b, 0, D, 0, F, 8)
        for j, b in enumerate(cfg['w4']): blocks['4', j] = (w4_hbm, w4b) + b
        sem_of = {k: wsem.at[i] for i, k in enumerate(blocks)}

        def geom(key):
            src, dst, r0, nr, c0, nc, rd = blocks[key]
            nd = nr // rd
            ns = max(s for s in range(1, cfg.get('ns4', cfg['ns']) + 1 if key[0] == '4' else cfg['ns'] + 1) if nd % s == 0)
            return ns, nd // ns
        def start(key, r, prio):
            src, dst, r0, nr, c0, nc, rd = blocks[key]
            pltpu.make_async_copy(src.at[pl.ds(r, rd), pl.ds(c0, nc)], dst.at[pl.ds(r, rd), pl.ds(c0, nc)],
                                  sem_of[key]).start(priority=prio)
        def wi(key, i0, i1):
            src, dst, r0, nr, c0, nc, rd = blocks[key]
            ns, per = geom(key)
            def it(i, _):
                for j in range(ns):
                    r = r0 + (j * per + i) * rd
                    if not isinstance(r, int):
                        r = pl.multiple_of(r, 8)
                    start(key, r, j % 2)
            if i1 - i0 > 1:
                lax.fori_loop(i0, i1, it, None)
            elif i1 > i0:
                it(i0, None)
        def descs(keys):
            out = []
            for k in keys:
                ns, per = geom(k)
                out += [(k, blocks[k][2] + (j * per + i) * blocks[k][6]) for i in range(per) for j in range(ns)]
            return out

        class Stream:
            def __init__(self, keys):
                self.groups = [(k, i) for k in keys for i in range(geom(k)[1])]
                self.pos = 0
            def upto(self, n):
                while self.pos < n:
                    k, i0 = self.groups[self.pos]
                    e = self.pos
                    while e < n and self.groups[e][0] == k: e += 1
                    wi(k, i0, i0 + e - self.pos)
                    self.pos = e
            def ahead(self, key, extra):
                last = max(i for i, g in enumerate(self.groups) if g[0] == key) + 1
                while last < len(self.groups) and extra >= geom(self.groups[last][0])[0]:
                    extra -= geom(self.groups[last][0])[0]; last += 1
                self.upto(last)
                return extra if last == len(self.groups) else 0

        class Static:
            def __init__(self, keys):
                d = descs(keys); lag = cfg['lag']
                mid = d[lag:len(d) - lag]
                p0 = d[:lag] + mid[0::2]
                p1 = mid[1::2] + d[len(d) - lag:]
                self.seq = [x for a, b in zip(p0, p1) for x in (a + (0,), b + (1,))]
                assert len(self.seq) == len(d)
                self.pos = 0
            def upto(self, n):
                n = min(n, len(self.seq))
                while self.pos < n:
                    start(*self.seq[self.pos]); self.pos += 1
            def ahead(self, key, extra):
                self.upto(max(i for i, g in enumerate(self.seq) if g[0] == key) + 1 + extra)

        def ww(key):
            src, dst, r0, nr, c0, nc, rd = blocks[key]
            v = dst.at[pl.ds(r0, nr), pl.ds(c0, nc)]
            pltpu.make_async_copy(v, v, sem_of[key]).wait()
        def kv_issue(src, dst, i, sem):
            for t in range(R // CH):
                r0 = i * R + t * CH
                for j, h in enumerate(cfg['perm']):
                    rs = SK - W + ((r0 + h * cfg['shift'] * CH) & (W - 1))
                    rd = r0
                    if not isinstance(r0, int):
                        rs, rd = pl.multiple_of(rs, CH), pl.multiple_of(rd, CH)
                    pltpu.make_async_copy(src.at[0, h, pl.ds(rs, CH)], dst.at[h, pl.ds(rd, CH)], sem).start(priority=j % 2)
        def kv_issue_range(src, dst, sems, i0, i1):
            def it(i, _):
                kv_issue(src, dst, i, sems.at[i])
            if i1 > i0:
                lax.fori_loop(i0, i1, it, None)
        def kv_wait(dst, i, sem):
            v = dst.at[:, pl.ds(pl.multiple_of(i * R, R), R)]
            pltpu.make_async_copy(v, v, sem).wait()

        xcp = pltpu.make_async_copy(x_hbm.at[0], xb, ssem.at[0])
        ccp = pltpu.make_async_copy(c_hbm, cb, ssem.at[1])
        row8 = lax.broadcasted_iota(jnp.int32, (8, 1), 0)
        A = cfg['ahead']
        per_blk = HKV * R // CH

        head = Stream([('m', j) for j in range(nm)] + [('q', 0), ('q', 1)])
        if cfg['solo']:
            d = descs([('m', 0)])
            for t, (k, r) in enumerate(d):
                start(k, r, 1 if t < cfg['solo'] else (t - cfg['solo']) % 2)
            head.pos = geom(('m', 0))[1]
        else:
            head.upto(6)
        ccp.start(); xcp.start()
        head.ahead(('m', nm - 1), A)
        ccp.wait(); xcp.wait()
        for j in range(nm): ww(('m', j))
        if do:
            c = jnp.broadcast_to(cb[...].astype(F32), (8, D))
            s = (c * jax.nn.sigmoid(c)).astype(BF)
            mod = jnp.dot(s, wmb[...], preferred_element_type=F32)
            for t in range(6):
                modb[t] = mod[:, D * t:D * (t + 1)]
            x = jnp.broadcast_to(xb[...].astype(F32), (8, D))
            h = (_ln(x) * (1.0 + modb[1]) + modb[0]).astype(BF)
        head.upto(len(head.groups))
        kv_issue_range(k_hbm, kb, ksem, 0, L)
        def q_step(j, _):
            src, dst = wq_hbm, wqb
            v = wqb.at[:, pl.ds(0, 2048)]
            pltpu.make_async_copy(v, v, wsem.at[nm + j]).wait()
            if do:
                r = jnp.dot(h, wqb[:, pl.ds(pl.multiple_of(2048 * j, 2048), 2048)], preferred_element_type=F32)
                q = r[:, 0:DH]
                for t in range(1, 8):
                    q = jnp.where(row8 == t, r[:, DH * t:DH * (t + 1)], q)
                qb[j] = q * (DH ** -0.5)
        lax.fori_loop(0, 2, q_step, None)
        if do:
            q = [qb[g].astype(BF) for g in range(2)]

        def k_step(i, mx):
            @pl.when(i + L < NB)
            def _():
                kv_issue(k_hbm, kb, i + L, ksem.at[i + L])
            @pl.when(i + L >= NB)
            def _():
                kv_issue(v_hbm, vb, i + L - NB, vsem.at[i + L - NB])
            kv_wait(kb, i, ksem.at[i])
            if not do or 'k' in skip:
                return mx
            r0 = pl.multiple_of(i * R, R)
            out = []
            for g in range(2):
                sg = None
                for j in range(4):
                    r = lax.dot_general(q[g], kb[4 * g + j, pl.ds(r0, R), :], NT, preferred_element_type=F32)
                    sg = r if sg is None else jnp.where(row8 // 2 == j, r, sg)
                sc[g, i] = sg
                m = sg[:, 0:128]
                for t in range(1, R // 128):
                    m = jnp.maximum(m, sg[:, 128 * t:128 * (t + 1)])
                out.append(jnp.maximum(mx[g], m))
            return tuple(out)
        ninf = jnp.full((8, 128), -jnp.inf, F32)
        mx = lax.fori_loop(0, NB, k_step, (ninf, ninf))

        if do:
            for g in range(2):
                m = jnp.max(mx[g], axis=-1, keepdims=True)
                e = jnp.exp(sc[g] - m)
                l = jnp.sum(jnp.sum(e, axis=0), axis=-1, keepdims=True)
                sc[g] = e * (1.0 / l)

        tail = Static([('o', 0), ('o', 1), ('3', 0)] + [('4', j) for j in range(n4)])
        def v_step(i, acc):
            @pl.when(i + L < NB)
            def _():
                kv_issue(v_hbm, vb, i + L, vsem.at[i + L])
            for t in range(L):
                @pl.when(i + L == NB + t)
                def _():
                    tail.upto((t + 1) * per_blk)
            kv_wait(vb, i, vsem.at[i])
            if not do or 'v' in skip:
                return acc
            r0 = pl.multiple_of(i * R, R)
            out = []
            for g in range(2):
                pg = sc[g, i].astype(BF)
                og = None
                for j in range(4):
                    r = jnp.dot(pg, vb[4 * g + j, pl.ds(r0, R), :], preferred_element_type=F32)
                    og = r if og is None else jnp.where(row8 // 2 == j, r, og)
                out.append(acc[g] + og)
            return tuple(out)
        z = jnp.zeros((8, DH), F32)
        o = lax.fori_loop(0, NB, v_step, (z, z))

        for j in range(2):
            tail.ahead(('o', j), cfg.get('tahead', A))
            ww(('o', j))
            if do:
                lhs = jnp.concatenate([jnp.where(row8 == t, o[j], 0.0) for t in range(8)], axis=1).astype(BF)
                accb[j] = lax.dot_general(lhs, wob[:, 2048 * j:2048 * (j + 1)], NT, preferred_element_type=F32)
        tail.upto(10 ** 6)
        if do:
            attn = jnp.sum(accb[0] + accb[1], axis=0, keepdims=True)
            x1 = x + modb[2] * attn
            h2 = _ln(x1) * (1.0 + modb[4]) + modb[3]
            hn = _ln(h2).astype(BF)
        ww(('3', 0))
        if cfg.get('probe') == -1: pl.delay(3000)
        if do:
            u = jax.nn.gelu(jnp.dot(hn, w3b[...], preferred_element_type=F32), approximate=True).astype(BF)
            gb = modb[5]
            res = x1 + gb * h2
        tiles = [(128 * t, min(128, D - 128 * t)) for t in range(4)]
        if do:
            rt = [res[:, a:a + n] for a, n in tiles]
            gt = [gb[:, a:a + n] for a, n in tiles]
        groups = cfg.get('w4wait') or [[j] for j in range(n4)]
        for grp in groups:
            for j in grp:
                ww(('4', j))
                if cfg.get('probe') == j: pl.delay(3000)
            if do and '4' not in skip:
                for j in grp:
                    r0, nr, c0, nc, _ = cfg['w4'][j]
                    y = lax.dot_general(u[:, c0:c0 + nc], w4b[r0:r0 + nr, c0:c0 + nc], NT, preferred_element_type=F32)
                    for t, (a, n) in enumerate(tiles):
                        if r0 <= a < r0 + nr:
                            rt[t] = rt[t] + gt[t] * y[:, a - r0:a - r0 + n]
        if do:
            ob[...] = jnp.concatenate([r[0:1, :] for r in rt], axis=1).astype(BF)
        else:
            ob[...] = jnp.zeros(ob.shape, BF)
        ocp = pltpu.make_async_copy(ob, o_hbm.at[0], ssem.at[2])
        ocp.start(priority=cfg.get('oprio', 0)); ocp.wait()

    def f(A_x, A_k_cache, A_v_cache, A_wq, A_wo, B_x, B_w1, B_w2, B_w3, B_w4, c, w_mod):
        hb = pl.BlockSpec(memory_space=pltpu.HBM)
        args = [A_x, c, A_k_cache, A_v_cache, w_mod, A_wq, A_wo.T, B_w3, B_w4.T]
        args = [pltpu.with_memory_space_constraint(a, pltpu.HBM) for a in args]
        return pl.pallas_call(kernel, in_specs=[hb] * 9, out_specs=hb,
            out_shape=jax.ShapeDtypeStruct((1, 1, D), BF),
            scratch_shapes=[pltpu.VMEM((1, D), BF), pltpu.VMEM((1, D), BF),
                pltpu.VMEM((HKV, W, DH), BF), pltpu.VMEM((HKV, W, DH), BF),
                pltpu.VMEM((D, 6 * D), BF), pltpu.VMEM((D, HQ * DH), BF), pltpu.VMEM((D, HQ * DH), BF),
                pltpu.VMEM((D, F), BF), pltpu.VMEM((D, F), BF),
                pltpu.VMEM((2, NB, 8, R), F32), pltpu.VMEM((6, 8, D), F32), pltpu.VMEM((2, 8, DH), F32),
                pltpu.VMEM((2, 8, D), F32), pltpu.VMEM((1, D), BF),
                pltpu.SemaphoreType.DMA((5 + n4 + nm,)), pltpu.SemaphoreType.DMA((NB,)), pltpu.SemaphoreType.DMA((NB,)),
                pltpu.SemaphoreType.DMA((3,))],
            compiler_params=pltpu.CompilerParams(vmem_limit_bytes=100 * 2**20, disable_bounds_checks=True, disable_semaphore_checks=True),
            name="adaln_decode",
        )(*args)
    return f


@jax.jit
def pallas_adaLN_cond__sliding_block_cached__mixer_s_mlp__decode_kernel(
    A_x, A_k_cache, A_v_cache, A_wq, A_wo, B_x, B_w1, B_w2, B_w3, B_w4, c, w_mod):
    return make(solo=32)(A_x, A_k_cache, A_v_cache, A_wq, A_wo, B_x, B_w1, B_w2, B_w3, B_w4, c, w_mod)
```

```python
import jax
import jax.numpy as jnp
from jax import lax
from jax.experimental import pallas as pl
from jax.experimental.pallas import tpu as pltpu

D, F = 448, 1792
HQ, HKV, DH = 16, 8, 256
SK, W = 65536, 4096
QCOLS = HQ * DH // 2

KEYS = 256
CHUNK = 64
NBLK = W // KEYS
BLK_DESCS = HKV * KEYS // CHUNK
AHEAD = 3
HEAD_SKEW = 2 * CHUNK
QUEUE_LAG = 28
W4_BLOCKS = ((0, 256, 4), (256, 128, 1), (384, 64, 1))

BF16, F32 = jnp.bfloat16, jnp.float32
NT = (((1,), (1,)), ((), ()))

SEM_MOD, SEM_Q, SEM_O, SEM_W3, SEM_W4 = 0, 1, 3, 5, 6


def _layernorm(x):
    d = x - jnp.mean(x, axis=-1, keepdims=True)
    return d * lax.rsqrt(jnp.mean(d * d, axis=-1, keepdims=True) + 1e-5)


def _interleave(items, streams):
    per = len(items) // streams
    assert per * streams == len(items)
    return [items[s * per + i] for i in range(per) for s in range(streams)]


def _kernel(x_hbm, c_hbm, k_hbm, v_hbm, wm_hbm, wq_hbm, wo_hbm, w3_hbm, w4_hbm, out_hbm,
            x_vm, c_vm, k_vm, v_vm, wm_vm, wq_vm, wo_vm, w3_vm, w4_vm,
            mod_vm, q_vm, p_vm, o_vm, attn_vm, out_vm, w_sem, k_sem, v_sem, io_sem):

    def start_tile(src, dst, sem, row, col, ncols, queue):
        sl = (pl.ds(row, 8), pl.ds(col, ncols))
        pltpu.make_async_copy(src.at[sl], dst.at[sl], w_sem.at[sem]).start(priority=queue)

    def tiles(src, dst, sem, row0, nrows, col, ncols, streams):
        return _interleave([(src, dst, sem, r, col, ncols) for r in range(row0, row0 + nrows, 8)], streams)

    def wait_filled(view, sem):
        pltpu.make_async_copy(view, view, sem).wait()

    def start_wq(j):
        def body(i, carry):
            for s in range(8):
                row = pl.multiple_of((s * (D // 64) + i) * 8, 8)
                start_tile(wq_hbm, wq_vm, SEM_Q + j, row, j * QCOLS, QCOLS, s % 2)
            return carry
        lax.fori_loop(0, D // 64, body, None)

    def start_kv(src, dst, sems, blk):
        for t in range(KEYS // CHUNK):
            row = blk * KEYS + t * CHUNK
            for h in range(HKV):
                src_row = pl.multiple_of(SK - W + ((row + h * HEAD_SKEW) & (W - 1)), CHUNK)
                pltpu.make_async_copy(src.at[0, h, pl.ds(src_row, CHUNK)],
                                      dst.at[h, pl.ds(pl.multiple_of(row, CHUNK), CHUNK)],
                                      sems.at[blk]).start(priority=h % 2)

    def block_rows(blk):
        return pl.ds(pl.multiple_of(blk * KEYS, KEYS), KEYS)

    def head_cols(j):
        return pl.ds(pl.multiple_of(j * QCOLS, QCOLS), QCOLS)

    landing = (tiles(wo_hbm, wo_vm, SEM_O, 0, D, 0, QCOLS, 8)
               + tiles(wo_hbm, wo_vm, SEM_O + 1, 0, D, QCOLS, QCOLS, 8)
               + tiles(w3_hbm, w3_vm, SEM_W3, 0, D, 0, F, 8))
    for j, (row0, nrows, streams) in enumerate(W4_BLOCKS):
        landing += tiles(w4_hbm, w4_vm, SEM_W4 + j, row0, nrows, 0, F, streams)
    middle = landing[QUEUE_LAG:-QUEUE_LAG]
    pairs = zip(landing[:QUEUE_LAG] + middle[0::2], middle[1::2] + landing[-QUEUE_LAG:], strict=True)
    tail = [d for a, b in pairs for d in (a + (0,), b + (1,))]

    def start_tail(lo, hi):
        for d in tail[lo:hi]:
            start_tile(*d)

    def tail_end(sem):
        return 1 + max(i for i, d in enumerate(tail) if d[2] == sem)

    row_id = lax.broadcasted_iota(jnp.int32, (8, 1), 0)

    x_copy = pltpu.make_async_copy(x_hbm.at[0], x_vm, io_sem.at[0])
    c_copy = pltpu.make_async_copy(c_hbm, c_vm, io_sem.at[1])
    first = tiles(wm_hbm, wm_vm, SEM_MOD, 0, D, 0, 1280, 8) + tiles(wm_hbm, wm_vm, SEM_MOD, 0, D, 1280, 6 * D - 1280, 8)
    for i, d in enumerate(first):
        start_tile(*d, 1 if i < QUEUE_LAG + 4 else i % 2)
    c_copy.start()
    x_copy.start()
    start_wq(0)
    c_copy.wait()
    x_copy.wait()
    wait_filled(wm_vm, w_sem.at[SEM_MOD])

    c = jnp.broadcast_to(c_vm[...].astype(F32), (8, D))
    mod = jnp.dot((c * jax.nn.sigmoid(c)).astype(BF16), wm_vm[...], preferred_element_type=F32)
    for t in range(6):
        mod_vm[t] = mod[:, t * D:(t + 1) * D]
    x = jnp.broadcast_to(x_vm[...].astype(F32), (8, D))
    h = (_layernorm(x) * (1.0 + mod_vm[1]) + mod_vm[0]).astype(BF16)

    start_wq(1)

    def start_k(i, carry):
        start_kv(k_hbm, k_vm, k_sem, i)
        return carry
    lax.fori_loop(0, AHEAD, start_k, None)

    def q_step(g, carry):
        wait_filled(wq_vm.at[:, head_cols(g)], w_sem.at[SEM_Q + g])
        r = jnp.dot(h, wq_vm[:, head_cols(g)], preferred_element_type=F32)
        q = r[:, 0:DH]
        for t in range(1, 8):
            q = jnp.where(row_id == t, r[:, t * DH:(t + 1) * DH], q)
        q_vm[g] = q * (DH ** -0.5)
        return carry
    lax.fori_loop(0, 2, q_step, None)
    q = [q_vm[g].astype(BF16) for g in range(2)]

    def k_step(i, row_max):
        @pl.when(i + AHEAD < NBLK)
        def _():
            start_kv(k_hbm, k_vm, k_sem, i + AHEAD)

        @pl.when(i + AHEAD >= NBLK)
        def _():
            start_kv(v_hbm, v_vm, v_sem, i + AHEAD - NBLK)

        wait_filled(k_vm.at[:, block_rows(i)], k_sem.at[i])
        new_max = []
        for g in range(2):
            s = None
            for j in range(4):
                r = lax.dot_general(q[g], k_vm[4 * g + j, block_rows(i), :], NT, preferred_element_type=F32)
                s = r if s is None else jnp.where(row_id // 2 == j, r, s)
            p_vm[g, i] = s
            m = row_max[g]
            for t in range(KEYS // 128):
                m = jnp.maximum(m, s[:, 128 * t:128 * (t + 1)])
            new_max.append(m)
        return tuple(new_max)

    neg_inf = jnp.full((8, 128), -jnp.inf, F32)
    row_max = lax.fori_loop(0, NBLK, k_step, (neg_inf, neg_inf))

    for g in range(2):
        e = jnp.exp(p_vm[g] - jnp.max(row_max[g], axis=-1, keepdims=True))
        total = jnp.sum(jnp.sum(e, axis=0), axis=-1, keepdims=True)
        p_vm[g] = e * (1.0 / total)

    def v_step(i, acc):
        @pl.when(i + AHEAD < NBLK)
        def _():
            start_kv(v_hbm, v_vm, v_sem, i + AHEAD)

        for t in range(AHEAD):
            @pl.when(i + AHEAD == NBLK + t)
            def _():
                start_tail(t * BLK_DESCS, (t + 1) * BLK_DESCS)

        wait_filled(v_vm.at[:, block_rows(i)], v_sem.at[i])
        new_acc = []
        for g in range(2):
            p = p_vm[g, i].astype(BF16)
            o = None
            for j in range(4):
                r = jnp.dot(p, v_vm[4 * g + j, block_rows(i), :], preferred_element_type=F32)
                o = r if o is None else jnp.where(row_id // 2 == j, r, o)
            new_acc.append(acc[g] + o)
        return tuple(new_acc)

    zero = jnp.zeros((8, DH), F32)
    o = lax.fori_loop(0, NBLK, v_step, (zero, zero))

    for g in range(2):
        o_vm[g] = jnp.concatenate([jnp.where(row_id == t, o[g], 0.0) for t in range(8)], axis=1)

    marks = (AHEAD * BLK_DESCS,
             tail_end(SEM_O) + AHEAD * BLK_DESCS,
             tail_end(SEM_O + 1) + AHEAD * BLK_DESCS)
    assert marks[-1] >= len(tail)

    def o_step(g, carry):
        for t in range(2):
            @pl.when(g == t)
            def _():
                start_tail(marks[t], marks[t + 1])

        wait_filled(wo_vm.at[:, head_cols(g)], w_sem.at[SEM_O + g])
        attn_vm[g] = lax.dot_general(o_vm[g].astype(BF16), wo_vm[:, head_cols(g)], NT, preferred_element_type=F32)
        return carry
    lax.fori_loop(0, 2, o_step, None)

    x1 = x + mod_vm[2] * jnp.sum(attn_vm[0] + attn_vm[1], axis=0, keepdims=True)
    h2 = _layernorm(x1) * (1.0 + mod_vm[4]) + mod_vm[3]
    h2_norm = _layernorm(h2).astype(BF16)

    wait_filled(w3_vm, w_sem.at[SEM_W3])
    u = jax.nn.gelu(jnp.dot(h2_norm, w3_vm[...], preferred_element_type=F32), approximate=True).astype(BF16)
    gate = mod_vm[5]
    base = x1 + gate * h2

    out = []
    for j, (row0, nrows, _) in enumerate(W4_BLOCKS):
        rows = pl.ds(row0, nrows)
        wait_filled(w4_vm.at[rows, :], w_sem.at[SEM_W4 + j])
        y = lax.dot_general(u, w4_vm[rows, :], NT, preferred_element_type=F32)
        out.append(base[:, row0:row0 + nrows] + gate[:, row0:row0 + nrows] * y)
    out_vm[...] = jnp.concatenate(out, axis=1)[0:1, :].astype(out_vm.dtype)

    out_copy = pltpu.make_async_copy(out_vm, out_hbm.at[0], io_sem.at[2])
    out_copy.start()
    out_copy.wait()


@jax.jit
def pallas_adaLN_cond__sliding_block_cached__mixer_s_mlp__decode_kernel(
    A_x: jax.Array,
    A_k_cache: jax.Array,
    A_v_cache: jax.Array,
    A_wq: jax.Array,
    A_wo: jax.Array,
    B_x: jax.Array,
    B_w1: jax.Array,
    B_w2: jax.Array,
    B_w3: jax.Array,
    B_w4: jax.Array,
    c: jax.Array,
    w_mod: jax.Array,
):
    del B_x, B_w1, B_w2
    assert A_x.shape == (1, 1, D) and A_k_cache.shape == A_v_cache.shape == (1, HKV, SK, DH)

    operands = [A_x, c, A_k_cache, A_v_cache, w_mod, A_wq, A_wo.T, B_w3, B_w4.T]
    operands = [pltpu.with_memory_space_constraint(a, pltpu.HBM) for a in operands]
    hbm = pl.BlockSpec(memory_space=pltpu.HBM)
    return pl.pallas_call(
        _kernel,
        in_specs=[hbm] * len(operands),
        out_specs=hbm,
        out_shape=jax.ShapeDtypeStruct((1, 1, D), A_x.dtype),
        scratch_shapes=[
            pltpu.VMEM((1, D), BF16),
            pltpu.VMEM((1, D), BF16),
            pltpu.VMEM((HKV, W, DH), BF16),
            pltpu.VMEM((HKV, W, DH), BF16),
            pltpu.VMEM((D, 6 * D), BF16),
            pltpu.VMEM((D, HQ * DH), BF16),
            pltpu.VMEM((D, HQ * DH), BF16),
            pltpu.VMEM((D, F), BF16),
            pltpu.VMEM((D, F), BF16),
            pltpu.VMEM((6, 8, D), F32),
            pltpu.VMEM((2, 8, DH), F32),
            pltpu.VMEM((2, NBLK, 8, KEYS), F32),
            pltpu.VMEM((2, 8, QCOLS), F32),
            pltpu.VMEM((2, 8, D), F32),
            pltpu.VMEM((1, D), BF16),
            pltpu.SemaphoreType.DMA((SEM_W4 + len(W4_BLOCKS),)),
            pltpu.SemaphoreType.DMA((NBLK,)),
            pltpu.SemaphoreType.DMA((NBLK,)),
            pltpu.SemaphoreType.DMA((3,)),
        ],
        compiler_params=pltpu.CompilerParams(
            vmem_limit_bytes=64 * 2**20,
            disable_semaphore_checks=True,
        ),
        name="adaln_decode",
    )(*operands)
```

```python
import jax
import jax.numpy as jnp
from jax import lax
from jax.experimental import pallas as pl
from jax.experimental.pallas import tpu as pltpu

D, F = 448, 1792
HQ, HKV, DH = 16, 8, 256
SK, W = 65536, 4096
QCOLS = HQ * DH // 2

KEYS = 256
CHUNK = 64
NBLK = W // KEYS
BLK_DESCS = HKV * KEYS // CHUNK
AHEAD = 3
HEAD_SKEW = 2 * CHUNK
QUEUE_LAG = 28
W3_SLACK = 4
W4_BLOCKS = ((0, 256), (256, 128), (384, 64))

BF16, F32 = jnp.bfloat16, jnp.float32
NT = (((1,), (1,)), ((), ()))

SEM_MOD, SEM_Q, SEM_O, SEM_W3, SEM_W4 = 0, 1, 3, 5, 6


def _layernorm(x):
    d = x - jnp.mean(x, axis=-1, keepdims=True)
    return d * lax.rsqrt(jnp.mean(d * d, axis=-1, keepdims=True) + 1e-5)


def _interleave(items, streams):
    per = len(items) // streams
    assert per * streams == len(items)
    return [items[s * per + i] for i in range(per) for s in range(streams)]


def _kernel(x_hbm, c_hbm, k_hbm, v_hbm, wm_hbm, wq_hbm, wo_hbm, w3_hbm, w4_hbm, out_hbm,
            x_vm, c_vm, k_vm, v_vm, wm_vm, wq_vm, wo_vm, w3_vm, w4_vm,
            mod_vm, q_vm, p_vm, o_vm, attn_vm, out_vm, w_sem, k_sem, v_sem, io_sem):

    def start_tile(src, dst, sem, row, col, ncols, queue):
        sl = (pl.ds(row, 8), pl.ds(col, ncols))
        pltpu.make_async_copy(src.at[sl], dst.at[sl], w_sem.at[sem]).start(priority=queue)

    def tiles(src, dst, sem, row0, nrows, col, ncols, streams):
        return _interleave([(src, dst, sem, r, col, ncols) for r in range(row0, row0 + nrows, 8)], streams)

    def wait_filled(view, sem):
        pltpu.make_async_copy(view, view, sem).wait()

    def start_wq(j):
        def body(i, carry):
            for s in range(8):
                row = pl.multiple_of((s * (D // 64) + i) * 8, 8)
                start_tile(wq_hbm, wq_vm, SEM_Q + j, row, j * QCOLS, QCOLS, s % 2)
            return carry
        lax.fori_loop(0, D // 64, body, None)

    def start_kv(src, dst, sems, blk):
        for t in range(KEYS // CHUNK):
            row = blk * KEYS + t * CHUNK
            for h in range(HKV):
                src_row = pl.multiple_of(SK - W + ((row + h * HEAD_SKEW) & (W - 1)), CHUNK)
                pltpu.make_async_copy(src.at[0, h, pl.ds(src_row, CHUNK)],
                                      dst.at[h, pl.ds(pl.multiple_of(row, CHUNK), CHUNK)],
                                      sems.at[blk]).start(priority=h % 2)

    def block_rows(blk):
        return pl.ds(pl.multiple_of(blk * KEYS, KEYS), KEYS)

    def head_cols(j):
        return pl.ds(pl.multiple_of(j * QCOLS, QCOLS), QCOLS)

    early = (tiles(wo_hbm, wo_vm, SEM_O, 0, D, 0, QCOLS, 8)
             + tiles(wo_hbm, wo_vm, SEM_O + 1, 0, D, QCOLS, QCOLS, 8)
             + tiles(w3_hbm, w3_vm, SEM_W3, 0, D, 0, F, 8))
    late = [d for j, (row0, nrows) in enumerate(W4_BLOCKS)
            for d in tiles(w4_hbm, w4_vm, SEM_W4 + j, row0, nrows, 0, F, 1)]
    late1 = QUEUE_LAG + W3_SLACK
    paired = len(early) - (2 * late1 - len(late))
    queue0 = early[0:paired:2] + early[paired:] + late[:-late1]
    queue1 = early[1:paired:2] + late[-late1:]
    tail = [d for a, b in zip(queue0, queue1, strict=True) for d in (a + (0,), b + (1,))]

    def start_tail(lo, hi):
        for d in tail[lo:hi]:
            start_tile(*d)

    def tail_end(sem):
        return 1 + max(i for i, d in enumerate(tail) if d[2] == sem)

    row_id = lax.broadcasted_iota(jnp.int32, (8, 1), 0)

    x_copy = pltpu.make_async_copy(x_hbm.at[0], x_vm, io_sem.at[0])
    c_copy = pltpu.make_async_copy(c_hbm, c_vm, io_sem.at[1])
    first = tiles(wm_hbm, wm_vm, SEM_MOD, 0, D, 0, 1280, 8) + tiles(wm_hbm, wm_vm, SEM_MOD, 0, D, 1280, 6 * D - 1280, 8)
    for i, d in enumerate(first):
        start_tile(*d, 1 if i < QUEUE_LAG + 4 else i % 2)
    c_copy.start()
    x_copy.start()
    start_wq(0)
    c_copy.wait()
    x_copy.wait()
    wait_filled(wm_vm, w_sem.at[SEM_MOD])

    c = jnp.broadcast_to(c_vm[...].astype(F32), (8, D))
    mod = jnp.dot((c * jax.nn.sigmoid(c)).astype(BF16), wm_vm[...], preferred_element_type=F32)
    for t in range(6):
        mod_vm[t] = mod[:, t * D:(t + 1) * D]
    x = jnp.broadcast_to(x_vm[...].astype(F32), (8, D))
    h = (_layernorm(x) * (1.0 + mod_vm[1]) + mod_vm[0]).astype(BF16)

    start_wq(1)

    def start_k(i, carry):
        start_kv(k_hbm, k_vm, k_sem, i)
        return carry
    lax.fori_loop(0, AHEAD, start_k, None)

    def q_step(g, carry):
        wait_filled(wq_vm.at[:, head_cols(g)], w_sem.at[SEM_Q + g])
        r = jnp.dot(h, wq_vm[:, head_cols(g)], preferred_element_type=F32)
        q = r[:, 0:DH]
        for t in range(1, 8):
            q = jnp.where(row_id == t, r[:, t * DH:(t + 1) * DH], q)
        q_vm[g] = q * (DH ** -0.5)
        return carry
    lax.fori_loop(0, 2, q_step, None)
    q = [q_vm[g].astype(BF16) for g in range(2)]

    def k_step(i, row_max):
        @pl.when(i + AHEAD < NBLK)
        def _():
            start_kv(k_hbm, k_vm, k_sem, i + AHEAD)

        @pl.when(i + AHEAD >= NBLK)
        def _():
            start_kv(v_hbm, v_vm, v_sem, i + AHEAD - NBLK)

        wait_filled(k_vm.at[:, block_rows(i)], k_sem.at[i])
        new_max = []
        for g in range(2):
            s = None
            for j in range(4):
                r = lax.dot_general(q[g], k_vm[4 * g + j, block_rows(i), :], NT, preferred_element_type=F32)
                s = r if s is None else jnp.where(row_id // 2 == j, r, s)
            p_vm[g, i] = s
            m = row_max[g]
            for t in range(KEYS // 128):
                m = jnp.maximum(m, s[:, 128 * t:128 * (t + 1)])
            new_max.append(m)
        return tuple(new_max)

    neg_inf = jnp.full((8, 128), -jnp.inf, F32)
    row_max = lax.fori_loop(0, NBLK, k_step, (neg_inf, neg_inf))

    for g in range(2):
        e = jnp.exp(p_vm[g] - jnp.max(row_max[g], axis=-1, keepdims=True))
        total = jnp.sum(jnp.sum(e, axis=0), axis=-1, keepdims=True)
        p_vm[g] = e * (1.0 / total)

    def v_step(i, acc):
        @pl.when(i + AHEAD < NBLK)
        def _():
            start_kv(v_hbm, v_vm, v_sem, i + AHEAD)

        for t in range(AHEAD):
            @pl.when(i + AHEAD == NBLK + t)
            def _():
                start_tail(t * BLK_DESCS, (t + 1) * BLK_DESCS)

        wait_filled(v_vm.at[:, block_rows(i)], v_sem.at[i])
        new_acc = []
        for g in range(2):
            p = p_vm[g, i].astype(BF16)
            o = None
            for j in range(4):
                r = jnp.dot(p, v_vm[4 * g + j, block_rows(i), :], preferred_element_type=F32)
                o = r if o is None else jnp.where(row_id // 2 == j, r, o)
            new_acc.append(acc[g] + o)
        return tuple(new_acc)

    zero = jnp.zeros((8, DH), F32)
    o = lax.fori_loop(0, NBLK, v_step, (zero, zero))

    for g in range(2):
        o_vm[g] = jnp.concatenate([jnp.where(row_id == t, o[g], 0.0) for t in range(8)], axis=1)

    marks = (AHEAD * BLK_DESCS, tail_end(SEM_O) + AHEAD * BLK_DESCS, len(tail))

    def o_step(g, carry):
        for t in range(2):
            @pl.when(g == t)
            def _():
                start_tail(marks[t], marks[t + 1])

        wait_filled(wo_vm.at[:, head_cols(g)], w_sem.at[SEM_O + g])
        attn_vm[g] = lax.dot_general(o_vm[g].astype(BF16), wo_vm[:, head_cols(g)], NT, preferred_element_type=F32)
        return carry
    lax.fori_loop(0, 2, o_step, None)

    x1 = x + mod_vm[2] * jnp.sum(attn_vm[0] + attn_vm[1], axis=0, keepdims=True)
    h2 = _layernorm(x1) * (1.0 + mod_vm[4]) + mod_vm[3]
    h2_norm = _layernorm(h2).astype(BF16)

    wait_filled(w3_vm, w_sem.at[SEM_W3])
    u = jax.nn.gelu(jnp.dot(h2_norm, w3_vm[...], preferred_element_type=F32), approximate=True).astype(BF16)
    gate = mod_vm[5]
    base = x1 + gate * h2

    out = []
    for j, (row0, nrows) in enumerate(W4_BLOCKS):
        rows = pl.ds(row0, nrows)
        wait_filled(w4_vm.at[rows, :], w_sem.at[SEM_W4 + j])
        y = lax.dot_general(u, w4_vm[rows, :], NT, preferred_element_type=F32)
        out.append(base[:, row0:row0 + nrows] + gate[:, row0:row0 + nrows] * y)
    out_vm[...] = jnp.concatenate(out, axis=1)[0:1, :].astype(out_vm.dtype)

    out_copy = pltpu.make_async_copy(out_vm, out_hbm.at[0], io_sem.at[2])
    out_copy.start()
    out_copy.wait()


@jax.jit
def pallas_adaLN_cond__sliding_block_cached__mixer_s_mlp__decode_kernel(
    A_x: jax.Array,
    A_k_cache: jax.Array,
    A_v_cache: jax.Array,
    A_wq: jax.Array,
    A_wo: jax.Array,
    B_x: jax.Array,
    B_w1: jax.Array,
    B_w2: jax.Array,
    B_w3: jax.Array,
    B_w4: jax.Array,
    c: jax.Array,
    w_mod: jax.Array,
):
    del B_x, B_w1, B_w2
    assert A_x.shape == (1, 1, D) and A_k_cache.shape == A_v_cache.shape == (1, HKV, SK, DH)

    operands = [A_x, c, A_k_cache, A_v_cache, w_mod, A_wq, A_wo.T, B_w3, B_w4.T]
    operands = [pltpu.with_memory_space_constraint(a, pltpu.HBM) for a in operands]
    hbm = pl.BlockSpec(memory_space=pltpu.HBM)
    return pl.pallas_call(
        _kernel,
        in_specs=[hbm] * len(operands),
        out_specs=hbm,
        out_shape=jax.ShapeDtypeStruct((1, 1, D), A_x.dtype),
        scratch_shapes=[
            pltpu.VMEM((1, D), BF16),
            pltpu.VMEM((1, D), BF16),
            pltpu.VMEM((HKV, W, DH), BF16),
            pltpu.VMEM((HKV, W, DH), BF16),
            pltpu.VMEM((D, 6 * D), BF16),
            pltpu.VMEM((D, HQ * DH), BF16),
            pltpu.VMEM((D, HQ * DH), BF16),
            pltpu.VMEM((D, F), BF16),
            pltpu.VMEM((D, F), BF16),
            pltpu.VMEM((6, 8, D), F32),
            pltpu.VMEM((2, 8, DH), F32),
            pltpu.VMEM((2, NBLK, 8, KEYS), F32),
            pltpu.VMEM((2, 8, QCOLS), F32),
            pltpu.VMEM((2, 8, D), F32),
            pltpu.VMEM((1, D), BF16),
            pltpu.SemaphoreType.DMA((SEM_W4 + len(W4_BLOCKS),)),
            pltpu.SemaphoreType.DMA((NBLK,)),
            pltpu.SemaphoreType.DMA((NBLK,)),
            pltpu.SemaphoreType.DMA((3,)),
        ],
        compiler_params=pltpu.CompilerParams(
            vmem_limit_bytes=64 * 2**20,
            disable_semaphore_checks=True,
        ),
        name="adaln_decode",
    )(*operands)
```
